```python
import jax
import jax.numpy as jnp

def _softmax(x, axis=-1):
    return jax.nn.softmax(x, axis=axis)
def _gelu(x):
    return jax.nn.gelu(x, approximate=True)
def _silu(x):
    return jax.nn.silu(x)
def _sigmoid(x):
    return jax.nn.sigmoid(x)
def _layernorm(x, axis=-1, eps=1e-5):
    m = jnp.mean(x, axis=axis, keepdims=True)
    v = jnp.var(x, axis=axis, keepdims=True)
    return (x - m) / jnp.sqrt(v + eps)
def _scatter_add(tgt, idx, src, axis=0):
    return tgt.at[idx].add(src)
def _segment_sum(src, seg, n):
    return jax.ops.segment_sum(src, seg, n)
class _Rng:
    def __init__(self, key):
        self._k = key
    def _next(self):
        self._k, sub = jax.random.split(self._k)
        return sub
    def normal(self, shape):
        return jax.random.normal(self._next(), shape, dtype=jnp.bfloat16)
    def randint(self, lo, hi, shape):
        return jax.random.randint(self._next(), shape, lo, hi, dtype=jnp.int32)
    def uniform(self, shape, lo=0.0, hi=1.0):
        return jax.random.uniform(self._next(), shape, jnp.bfloat16, lo, hi)
    def permutation(self, n):
        return jax.random.permutation(self._next(), n)


kernel_name = 'recurrent_scan__mha_block_cached__moe_arch_mod__prompt'

def setup_inputs():
    _rng = _Rng(jax.random.key(int.from_bytes(__import__("os").urandom(4), "little")))
    _w = (lambda a: (lambda t: t.astype(jnp.bfloat16) if jnp.issubdtype(t.dtype, jnp.floating) else t)(jnp.asarray(a)))
    def _A_setup():
        B, Sq, D = 1, 2048, 640
        H, Sk, Dh = 32, 2048, 128
        return {
            "x": _w((lambda *s: _rng.normal(s) * 0.05)(B, Sq, D)),
            "k_cache": _w((lambda *s: _rng.normal(s) * 0.05)(B, H, Sk, Dh)),
            "v_cache": _w((lambda *s: _rng.normal(s) * 0.05)(B, H, Sk, Dh)),
            "wq": _w((lambda *s: _rng.normal(s) * 0.05)(D, H * Dh) * (D ** -0.5)),
            "wo": _w((lambda *s: _rng.normal(s) * 0.05)(H * Dh, D) * ((H * Dh) ** -0.5)),
        }
    _A_in = _A_setup()

    def _B_setup():
        B, S, D, F, C = 1, 2048, 640, 1728, 8
        return {
            "x": _w((lambda *s: _rng.normal(s) * 0.05)(B, S, D)),
            "w_r": _w((lambda *s: _rng.normal(s) * 0.05)(D)),
            "w_gate": _w((lambda *s: _rng.normal(s) * 0.05)(D, F)),
            "w_up": _w((lambda *s: _rng.normal(s) * 0.05)(D, F)),
            "w_down": _w((lambda *s: _rng.normal(s) * 0.05)(F, D)),
        }
    _B_in = _B_setup()

    return {
        "A_x": _A_in["x"],
        "A_k_cache": _A_in["k_cache"],
        "A_v_cache": _A_in["v_cache"],
        "A_wq": _A_in["wq"],
        "A_wo": _A_in["wo"],
        "B_x": _B_in["x"],
        "B_w_r": _B_in["w_r"],
        "B_w_gate": _B_in["w_gate"],
        "B_w_up": _B_in["w_up"],
        "B_w_down": _B_in["w_down"],
    }

def reference(A_x, A_k_cache, A_v_cache, A_wq, A_wo, B_x, B_w_r, B_w_gate, B_w_up, B_w_down):
    def _A_ref(x, k_cache, v_cache, wq, wo):
        B, Sq, D = x.shape
        H, Dh = 32, 128
        q = (lambda x, *d: x.transpose(*d))((x @ wq).reshape(B, Sq, H, Dh), 0, 2, 1, 3)
        scores = jnp.einsum("bhqd,bhkd->bhqk", q, k_cache) * (Dh ** -0.5)
        p = _softmax(scores, axis=-1)
        o = jnp.einsum("bhqk,bhkd->bhqd", p, v_cache)
        return (lambda x, *d: x.transpose(*d))(o, 0, 2, 1, 3).reshape(B, Sq, H * Dh) @ wo

    def _B_ref(x, w_r, w_gate, w_up, w_down):
        B, S, D = x.shape
        C = 8
        r = x @ w_r
        idx = jnp.argsort(-r, axis=-1)[:, :C]
        idx_e = jnp.repeat(idx.reshape(B, C, 1), D, axis=2)
        x_sel = jnp.take_along_axis(x, idx_e, axis=1)
        g = _silu(x_sel @ w_gate)
        u = x_sel @ w_up
        y = (g * u) @ w_down
        r_sel = _sigmoid(jnp.take_along_axis(r, idx, axis=1))
        y = y * r_sel.reshape(B, C, 1)
        b_off = (jnp.arange(B) * S).reshape(B, 1)
        flat_idx = (idx + b_off).reshape(B * C)
        zero = (x * 0.0).reshape(B * S, D)
        upd = _scatter_add(zero, flat_idx, y.reshape(B * C, D), axis=0)
        return x + upd.reshape(B, S, D)

    x = A_x
    xn = _layernorm(x, axis=-1)
    s = _A_ref(xn, A_k_cache, A_v_cache, A_wq, A_wo)
    g = _silu(_B_ref(xn, B_w_r, B_w_gate, B_w_up, B_w_down))
    return x + s * g
```

```python
import jax
import jax.numpy as jnp
import ml_dtypes
import numpy as np
from jax import lax
import jax.experimental.pallas as pl
import jax.experimental.pallas.tpu as pltpu

S, D, H, DH, F, C = 2048, 640, 32, 128, 1728, 8
BQ = 256
CK = 512
RB = 256
HG = 4
OB = 256
HPB = 1
KVP = 2
bf16, f32, i32 = jnp.bfloat16, jnp.float32, jnp.int32
NT = (((1,), (1,)), ((), ()))
QSCALE = float(DH ** -0.5 * np.log2(np.e))
EPS = float(np.asarray(1e-5, ml_dtypes.bfloat16))
KEY_BASE = 0x20000000
X_PIECES = ((0, 256), (256, 256), (512, 512), (1024, 1024))
WQ_PIECES = ((0, 1), (1, 3), (4, 4))


def _round(v):
    return v.astype(bf16).astype(f32)


def _sigmoid(v):
    return 1.0 / (1.0 + jnp.exp(-v))


def _attention(heads, q_ref, k_ref, v_ref, o_ref, always):
    nb, nc, nt = S // BQ, S // CK, CK // 128
    scores, run_max, row_max, run_sum, acc = {}, {}, {}, {}, {}
    pace = []

    def qk(b, c):
        h, i = b
        s = lax.dot_general(q_ref[heads[h], i * BQ:(i + 1) * BQ, :], k_ref[heads[h], c * CK:(c + 1) * CK, :],
                            NT, preferred_element_type=f32)
        scores[b, c] = s
        m = run_max.get(b)
        for t in range(nt):
            st = s[:, t * 128:(t + 1) * 128]
            m = st if m is None else jnp.maximum(m, st)
        run_max[b] = m
        if c == nc - 1:
            row_max[b] = jnp.broadcast_to(jnp.max(m, axis=-1, keepdims=True), (BQ, 128))

    def pv(b, c):
        h, i = b
        m = row_max[b]
        if pace:
            m = jnp.where(always, m, pace.pop())
        s = scores.pop((b, c))
        ps = [jnp.exp2(s[:, t * 128:(t + 1) * 128] - m) for t in range(nt)]
        l = run_sum.get(b)
        for pt in ps:
            l = pt if l is None else l + pt
        run_sum[b] = l
        ps[-1] = jnp.where(always, ps[-1], l)
        p = jnp.concatenate(ps, axis=1).astype(bf16)
        d = jnp.dot(p, v_ref[heads[h], c * CK:(c + 1) * CK, :], preferred_element_type=f32)
        o = d if c == 0 else acc[b] + d
        acc[b] = o
        if c == nc - 1:
            lr = jnp.sum(l, axis=-1, keepdims=True)
            r = pl.reciprocal(lr, approx=True)
            o = o * (r * (2.0 - lr * r))
            o_ref[heads[h], i * BQ:(i + 1) * BQ, :] = o.astype(bf16)
        pace.append(o)

    blocks = [(h, i) for h in range(len(heads)) for i in range(nb)]
    for c in range(nc):
        qk(blocks[0], c)
    for n, b in enumerate(blocks):
        for c in range(nc):
            if n + 1 < len(blocks):
                qk(blocks[n + 1], c)
            pv(b, c)


def _kernel(x_hbm, k_hbm, v_hbm, wq_hbm, wo_hbm, wr_hbm, wg_hbm, wu_hbm, wd_hbm, out_hbm,
            x_ref, k_ref, v_ref, wq_ref, wo_ref, wr_ref, wg_ref, wu_ref, wd_ref,
            xn_ref, xb_ref, r_ref, q_ref, oh_ref, res_ref, idx_ref, xsel_ref, rsel_ref,
            x_sem, wq_sem, kv_sem, w_sem, out_sem):
    cw = HG * DH
    x_cp = [pltpu.make_async_copy(x_hbm.at[pl.ds(a, n)], x_ref.at[pl.ds(a, n)], x_sem.at[j])
            for j, (a, n) in enumerate(X_PIECES)]
    wq_cp = [pltpu.make_async_copy(wq_hbm.at[:, pl.ds(a * cw, n * cw)], wq_ref.at[:, pl.ds(a * cw, n * cw)], wq_sem.at[j])
             for j, (a, n) in enumerate(WQ_PIECES)]
    hp = H // KVP
    k_cp = [pltpu.make_async_copy(k_hbm.at[pl.ds(j * hp, hp)], k_ref.at[pl.ds(j * hp, hp)], kv_sem.at[0, j]) for j in range(KVP)]
    v_cp = [pltpu.make_async_copy(v_hbm.at[pl.ds(j * hp, hp)], v_ref.at[pl.ds(j * hp, hp)], kv_sem.at[1, j]) for j in range(KVP)]
    wr_cp, wg_cp, wu_cp, wd_cp, wo_cp = [
        pltpu.make_async_copy(src, dst, w_sem.at[j]) for j, (src, dst) in enumerate(
            ((wr_hbm, wr_ref), (wg_hbm, wg_ref), (wu_hbm, wu_ref), (wd_hbm, wd_ref), (wo_hbm, wo_ref)))]

    def layernorm(rb):
        rows = slice(rb * RB, (rb + 1) * RB)
        x = x_ref[rows, :].astype(f32)
        mean = jnp.sum(x, axis=-1, keepdims=True) * (1.0 / D)
        xc = x - mean
        var = jnp.sum(xc * xc, axis=-1, keepdims=True) * (1.0 / D)
        den = _round(jnp.sqrt(_round(_round(var) + EPS)))
        xn = (_round(x - _round(mean)) * (1.0 / den)).astype(bf16)
        xn_ref[rows, :] = xn
        xb_ref[rows, :] = xn

    def router(rb):
        rows = slice(rb * RB, (rb + 1) * RB)
        r = jnp.sum(xn_ref[rows, :].astype(f32) * wr_ref[...].astype(f32), axis=-1, keepdims=True)
        eye = lax.broadcasted_iota(i32, (128, 128), 0) == lax.broadcasted_iota(i32, (128, 128), 1)
        for j in range(RB // 128):
            g = rb * (RB // 128) + j
            r_ref[g:g + 1, :] = jnp.sum(jnp.where(eye, r[j * 128:(j + 1) * 128], 0.0), axis=0, keepdims=True)

    def qproj(rb, g):
        rows = slice(rb * RB, (rb + 1) * RB)
        cols = g * cw if isinstance(g, int) else pl.multiple_of(g * cw, cw)
        q = jnp.dot(xn_ref[rows, :], wq_ref[:, pl.ds(cols, cw)], preferred_element_type=f32) * QSCALE
        for j in range(HG):
            q_ref[g * HG + j, rows, :] = q[:, j * DH:(j + 1) * DH].astype(bf16)

    def select_tokens():
        r = _round(r_ref[...])
        pos = lax.broadcasted_iota(i32, r.shape, 0) * 128 + lax.broadcasted_iota(i32, r.shape, 1)
        b = lax.shift_right_logical(pltpu.bitcast(jnp.where(r == 0.0, 0.0, r), i32), 16)
        u = jnp.where(b < 0x8000, b + 0x8000, 0xFFFF - b)
        u = jnp.where(r != r, 0, u)
        key = pltpu.bitcast(KEY_BASE + u * S + (S - 1 - pos), f32)
        sub8 = lax.broadcasted_iota(i32, (C, 128), 0)
        top_all = jnp.zeros((C, 128), f32)
        for c in range(C):
            top = jnp.max(jnp.max(key, axis=0, keepdims=True), axis=1, keepdims=True)
            key = jnp.where(key == top, 0.0, key)
            top_all = jnp.where(sub8 == c, top, top_all)
        bits = pltpu.bitcast(top_all, i32) - KEY_BASE
        u = lax.shift_right_logical(bits, 11)
        b = jnp.where(u >= 0x8000, u - 0x8000, 0xFFFF - u)
        rsel_ref[...] = _sigmoid(pltpu.bitcast(lax.shift_left(b, 16), f32))
        idx = (S - 1) - (bits & (S - 1))
        sub16 = lax.broadcasted_iota(i32, (16, D), 0)
        xsel = jnp.zeros((16, D), f32)
        for c in range(C):
            t = idx[c, 0]
            idx_ref[c] = t
            blk = xn_ref[pl.ds(pl.multiple_of(t & ~15, 16), 16), :].astype(f32)
            row = jnp.sum(jnp.where(sub16 == (t & 15), blk, 0.0), axis=0, keepdims=True)
            xsel = jnp.where(sub16 == c, row, xsel)
        xsel_ref[...] = xsel.astype(bf16)

    def ffn():
        xsel = xsel_ref[...]
        a = lax.dot_general(xsel, wg_ref[...], NT, preferred_element_type=f32)
        u = lax.dot_general(xsel, wu_ref[...], NT, preferred_element_type=f32)
        y = jnp.dot((a * _sigmoid(a) * u).astype(bf16), wd_ref[...], preferred_element_type=f32)
        y = _round(y[:C] * rsel_ref[:, :1])
        sub16 = lax.broadcasted_iota(i32, (16, D), 0)
        for c in range(C):
            t = idx_ref[c]
            rows = pl.ds(pl.multiple_of(t & ~15, 16), 16)
            blk = xb_ref[rows, :].astype(f32)
            xb_ref[rows, :] = jnp.where(sub16 == (t & 15), blk + y[c:c + 1], blk).astype(bf16)

    nrb = S // RB
    x_cp[0].start(); wq_cp[0].start(); x_cp[1].start(); x_cp[2].start(); x_cp[3].start()
    x_cp[0].wait()
    layernorm(0)
    wr_cp.start(); wq_cp[1].start()
    wq_cp[0].wait(); x_cp[1].wait()
    layernorm(1); qproj(0, 0)
    x_cp[2].wait()
    layernorm(2); qproj(1, 0); layernorm(3); qproj(2, 0)
    wq_cp[2].start(); wg_cp.start(); wu_cp.start(); wd_cp.start()
    x_cp[3].wait()
    for rb in range(3, nrb):
        if rb + 1 < nrb:
            layernorm(rb + 1)
        qproj(rb, 0)
    k_cp[0].start(); v_cp[0].start()
    wq_cp[1].wait(); wr_cp.wait()
    for rb in range(nrb):
        router(rb); qproj(rb, 1)
    select_tokens()
    for rb in range(nrb):
        qproj(rb, 2)
    wg_cp.wait(); wu_cp.wait(); wd_cp.wait()
    ffn()
    for rb in range(nrb):
        qproj(rb, 3)
    for j in range(1, KVP):
        k_cp[j].start(); v_cp[j].start()
    wo_cp.start()
    wq_cp[2].wait()

    def qproj_body(g, _):
        for rb in range(nrb):
            qproj(rb, g)
    lax.fori_loop(4, H // HG, qproj_body, None)

    def head_body(n, _):
        h = n * HPB
        for j in range(KVP):
            @pl.when(h == j * hp)
            def _():
                k_cp[j].wait(); v_cp[j].wait()
        _attention([h + j for j in range(HPB)], q_ref, k_ref, v_ref, oh_ref, h < H)
    lax.fori_loop(0, H // HPB, head_body, None)

    wo_cp.wait()

    def out_cp(i):
        rows = pl.ds(pl.multiple_of(i * OB, OB), OB)
        return pltpu.make_async_copy(res_ref.at[rows], out_hbm.at[rows], out_sem.at[i])

    def out_body(i, _):
        rows = pl.ds(pl.multiple_of(i * OB, OB), OB)
        s = None
        for g in range(H // HG):
            o = jnp.concatenate([oh_ref[g * HG + j, rows, :] for j in range(HG)], axis=1)
            d = jnp.dot(o, wo_ref[g * cw:(g + 1) * cw, :], preferred_element_type=f32)
            s = d if s is None else s + d
        xb = xb_ref[rows, :].astype(f32)
        res_ref[rows, :] = (x_ref[rows, :].astype(f32) + s * (xb * _sigmoid(xb))).astype(bf16)
        out_cp(i).start()
    lax.fori_loop(0, S // OB, out_body, None)
    for i in range(S // OB):
        out_cp(i).wait()


@jax.jit
def pallas_recurrent_scan__mha_block_cached__moe_arch_mod__prompt_kernel(
        A_x, A_k_cache, A_v_cache, A_wq, A_wo, B_x, B_w_r, B_w_gate, B_w_up, B_w_down):
    hbm = pl.BlockSpec(memory_space=pltpu.HBM)
    vm = pltpu.VMEM
    dma = pltpu.SemaphoreType.DMA
    out = pl.pallas_call(
        _kernel,
        in_specs=[hbm] * 9,
        out_specs=hbm,
        out_shape=jax.ShapeDtypeStruct((S, D), bf16),
        scratch_shapes=[
            vm((S, D), bf16), vm((H, S, DH), bf16), vm((H, S, DH), bf16), vm((D, H * DH), bf16), vm((H * DH, D), bf16),
            vm((1, D), bf16), vm((F, D), bf16), vm((F, D), bf16), vm((F, D), bf16),
            vm((S, D), bf16), vm((S, D), bf16), vm((S // 128, 128), f32), vm((H, S, DH), bf16), vm((H, S, DH), bf16),
            vm((S, D), bf16), pltpu.SMEM((C,), i32), vm((16, D), bf16), vm((C, 128), f32),
            dma((len(X_PIECES),)), dma((len(WQ_PIECES),)), dma((2, KVP)), dma((5,)), dma((S // OB,)),
        ],
        compiler_params=pltpu.CompilerParams(vmem_limit_bytes=120 * 2**20),
    )(A_x.reshape(S, D), A_k_cache.reshape(H, S, DH), A_v_cache.reshape(H, S, DH), A_wq, A_wo,
      B_w_r.reshape(1, D), B_w_gate.T, B_w_up.T, B_w_down)
    return out.reshape(1, S, D)
```

```python
import contextlib
import jax
import jax.numpy as jnp
import ml_dtypes
import numpy as np
from jax import lax
import jax.experimental.pallas as pl
import jax.experimental.pallas.tpu as pltpu

S, D, H, DH, F, C = 2048, 640, 32, 128, 1728, 8
BQ = 256
CK = 512
RB = 256
HG = 4
NG = H // HG
OB = 256
HPB = 2
FP = 256
PROF = 0
bf16, f32, i32 = jnp.bfloat16, jnp.float32, jnp.int32
NT = (((1,), (1,)), ((), ()))
QSCALE = float(DH ** -0.5 * np.log2(np.e))
EPS = float(np.asarray(1e-5, ml_dtypes.bfloat16))
KEY_BASE = 0x20000000
X_PIECES = ((0, 256), (256, 256), (512, 512), (1024, 1024))


def ns(name):
    return jax.named_scope(name) if PROF else contextlib.nullcontext()


def _round(v):
    return v.astype(bf16).astype(f32)


def _sigmoid(v):
    return 1.0 / (1.0 + jnp.exp(-v))


def _attention(heads, q_ref, k_ref, v_ref, o_ref, always):
    nb, nc, nt = S // BQ, S // CK, CK // 128
    scores, run_max, row_max, run_sum, acc = {}, {}, {}, {}, {}
    pace = []

    def qk(b, c):
        h, i = b
        s = lax.dot_general(q_ref[heads[h], i * BQ:(i + 1) * BQ, :], k_ref[h, c * CK:(c + 1) * CK, :],
                            NT, preferred_element_type=f32)
        scores[b, c] = s
        m = run_max.get(b)
        for t in range(nt):
            st = s[:, t * 128:(t + 1) * 128]
            m = st if m is None else jnp.maximum(m, st)
        run_max[b] = m
        if c == nc - 1:
            row_max[b] = jnp.broadcast_to(jnp.max(m, axis=-1, keepdims=True), (BQ, 128))

    def pv(b, c):
        h, i = b
        m = row_max[b]
        if pace:
            m = jnp.where(always, m, pace.pop())
        s = scores.pop((b, c))
        ps = [jnp.exp2(s[:, t * 128:(t + 1) * 128] - m) for t in range(nt)]
        l = run_sum.get(b)
        for pt in ps:
            l = pt if l is None else l + pt
        run_sum[b] = l
        ps[-1] = jnp.where(always, ps[-1], l)
        p = jnp.concatenate(ps, axis=1).astype(bf16)
        d = jnp.dot(p, v_ref[h, c * CK:(c + 1) * CK, :], preferred_element_type=f32)
        o = d if c == 0 else acc[b] + d
        acc[b] = o
        if c == nc - 1:
            lr = jnp.sum(l, axis=-1, keepdims=True)
            r = pl.reciprocal(lr, approx=True)
            o = o * (r * (2.0 - lr * r))
            o_ref[heads[h], i * BQ:(i + 1) * BQ, :] = o.astype(bf16)
        pace.append(o)

    blocks = [(h, i) for h in range(len(heads)) for i in range(nb)]
    for c in range(nc):
        qk(blocks[0], c)
    for n, b in enumerate(blocks):
        for c in range(nc):
            if n + 1 < len(blocks):
                qk(blocks[n + 1], c)
            pv(b, c)


def _kernel(x_hbm, k_hbm, v_hbm, wq_hbm, wo_hbm, wr_hbm, wg_hbm, wu_hbm, wd_hbm, out_hbm,
            x_ref, k_ref, v_ref, wq_ref, wo_ref, wr_ref, wgu_ref, wd_ref,
            xn_ref, xb_ref, r_ref, q_ref, oh_ref, res_ref, idx_ref, xsel_ref, rsel_ref, y_ref,
            x_sem, wr_sem, w_sem, kv_sem, out_sem):
    cw = HG * DH
    x_cp = [pltpu.make_async_copy(x_hbm.at[pl.ds(a, n)], x_ref.at[pl.ds(a, n)], x_sem.at[j])
            for j, (a, n) in enumerate(X_PIECES)]
    wr_cp = pltpu.make_async_copy(wr_hbm, wr_ref, wr_sem)

    def wq_cp(g):
        cols = g * cw if isinstance(g, int) else pl.multiple_of(g * cw, cw)
        return pltpu.make_async_copy(wq_hbm.at[:, pl.ds(cols, cw)], wq_ref.at[g], w_sem.at[0, g])

    def ffn_start(g):
        return min((g - 1) * FP, F - FP) if isinstance(g, int) else pl.multiple_of(jnp.minimum((g - 1) * FP, F - FP), 16)

    def chunk_cps(g):
        rows = pl.ds(ffn_start(g), FP)
        return (wq_cp(g),
                pltpu.make_async_copy(wg_hbm.at[rows], wgu_ref.at[g - 1, pl.ds(0, FP)], w_sem.at[1, g]),
                pltpu.make_async_copy(wu_hbm.at[rows], wgu_ref.at[g - 1, pl.ds(FP, FP)], w_sem.at[2, g]),
                pltpu.make_async_copy(wd_hbm.at[rows], wd_ref.at[g - 1], w_sem.at[3, g]))

    def head_cps(n):
        hs = pl.ds(n * HPB, HPB)
        wo_rows = pl.ds(pl.multiple_of(n * HPB * DH, DH), HPB * DH)
        return (pltpu.make_async_copy(k_hbm.at[hs], k_ref.at[n % 2], kv_sem.at[0, n]),
                pltpu.make_async_copy(v_hbm.at[hs], v_ref.at[n % 2], kv_sem.at[1, n]),
                pltpu.make_async_copy(wo_hbm.at[wo_rows], wo_ref.at[wo_rows], kv_sem.at[2, n]))

    def layernorm(r0, n=RB):
        rows = slice(r0, r0 + n)
        x = x_ref[rows, :].astype(f32)
        mean = jnp.sum(x, axis=-1, keepdims=True) * (1.0 / D)
        xc = x - mean
        var = jnp.sum(xc * xc, axis=-1, keepdims=True) * (1.0 / D)
        var = _round(_round(var) + EPS)
        rs = lax.rsqrt(var)
        den = _round(var * rs)
        xn32 = xc * (rs * (2.0 - den * rs))
        xn = xn32.astype(bf16)
        xn_ref[rows, :] = xn
        xb_ref[rows, :] = xn
        r = jnp.sum(xn32 * wr_ref[...].astype(f32).reshape(1, D), axis=-1, keepdims=True)
        eye = lax.broadcasted_iota(i32, (128, 128), 0) == lax.broadcasted_iota(i32, (128, 128), 1)
        for j in range(n // 128):
            g = r0 // 128 + j
            r_ref[g:g + 1, :] = jnp.sum(jnp.where(eye, r[j * 128:(j + 1) * 128], 0.0), axis=0, keepdims=True)

    def qproj(r0, g, n=RB):
        rows = slice(r0, r0 + n)
        q = jnp.dot(xn_ref[rows, :], wq_ref[g], preferred_element_type=f32) * QSCALE
        for j in range(HG):
            q_ref[g * HG + j, rows, :] = q[:, j * DH:(j + 1) * DH].astype(bf16)

    def select_tokens():
        r = _round(r_ref[...])
        pos = lax.broadcasted_iota(i32, r.shape, 0) * 128 + lax.broadcasted_iota(i32, r.shape, 1)
        b = lax.shift_right_logical(pltpu.bitcast(jnp.where(r == 0.0, 0.0, r), i32), 16)
        u = jnp.where(b < 0x8000, b + 0x8000, 0xFFFF - b)
        u = jnp.where(r != r, 0, u)
        key = pltpu.bitcast(KEY_BASE + u * S + (S - 1 - pos), f32)
        sub8 = lax.broadcasted_iota(i32, (C, 128), 0)
        top_all = jnp.zeros((C, 128), f32)
        for c in range(C):
            top = jnp.max(jnp.max(key, axis=0, keepdims=True), axis=1, keepdims=True)
            key = jnp.where(key == top, 0.0, key)
            top_all = jnp.where(sub8 == c, top, top_all)
        bits = pltpu.bitcast(top_all, i32) - KEY_BASE
        u = lax.shift_right_logical(bits, 11)
        b = jnp.where(u >= 0x8000, u - 0x8000, 0xFFFF - u)
        rsel_ref[...] = _sigmoid(pltpu.bitcast(lax.shift_left(b, 16), f32))
        idx = (S - 1) - (bits & (S - 1))
        sub16 = lax.broadcasted_iota(i32, (16, D), 0)
        xsel = jnp.zeros((16, D), f32)
        for c in range(C):
            t = idx[c, 0]
            idx_ref[c] = t
            blk = xn_ref[pl.ds(pl.multiple_of(t & ~15, 16), 16), :].astype(f32)
            row = jnp.sum(jnp.where(sub16 == (t & 15), blk, 0.0), axis=0, keepdims=True)
            xsel = jnp.where(sub16 == c, row, xsel)
        xsel_ref[...] = xsel.astype(bf16)
        y_ref[...] = jnp.zeros_like(y_ref)

    def scatter():
        y = _round(y_ref[:C, :] * rsel_ref[:, :1])
        sub16 = lax.broadcasted_iota(i32, (16, D), 0)
        for c in range(C):
            t = idx_ref[c]
            rows = pl.ds(pl.multiple_of(t & ~15, 16), 16)
            blk = xb_ref[rows, :].astype(f32)
            xb_ref[rows, :] = jnp.where(sub16 == (t & 15), blk + y[c:c + 1], blk).astype(bf16)

    nrb = S // RB
    with ns("p0_start"):
        x_cp[0].start(); wr_cp.start(); wq_cp(0).start()
        x_cp[0].wait(); wr_cp.wait()
        x_cp[1].start()
    with ns("p1_ln0"):
        layernorm(0)
    with ns("p2_wait"):
        wq_cp(0).wait()
        x_cp[2].start()
    with ns("p3a"):
        qproj(0, 0, 128)
    with ns("p3a_wait"):
        x_cp[1].wait()
        x_cp[3].start()
    with ns("p3b"):
        layernorm(256); qproj(128, 0, 128)
    with ns("p4_wait"):
        x_cp[2].wait()
        for cp in chunk_cps(1):
            cp.start()
    with ns("p5"):
        layernorm(512); qproj(256, 0); layernorm(768); qproj(512, 0)
    with ns("p6_wait"):
        x_cp[3].wait()
    with ns("p7"):
        layernorm(1024); qproj(768, 0); layernorm(1280); qproj(1024, 0); layernorm(1536); layernorm(1792); qproj(1280, 0)
        select_tokens()
        qproj(1536, 0); qproj(1792, 0)

    def qproj_body(g, _):
        @pl.when(g + 1 < NG)
        def _():
            for cp in chunk_cps(g + 1):
                cp.start()

        @pl.when(g + 1 == NG)
        def _():
            for cp in head_cps(0):
                cp.start()
        for cp in chunk_cps(g):
            cp.wait()
        with ns("pd_q"):
            au = None
            for rb in range(nrb):
                qproj(rb * RB, g)
                if rb < D // 128:
                    cols = slice(rb * 128, (rb + 1) * 128)
                    d = lax.dot_general(xsel_ref[:, cols], wgu_ref[g - 1, :, cols], NT, preferred_element_type=f32)
                    au = d if au is None else au + d
                elif rb == D // 128:
                    a, u = au[:, :FP], au[:, FP:]
                    fresh = lax.broadcasted_iota(i32, (16, FP), 1) >= (g - 1) * FP - ffn_start(g)
                    hid = jnp.where(fresh, a * _sigmoid(a) * u, 0.0).astype(bf16)
                    y_ref[...] += jnp.dot(hid, wd_ref[g - 1], preferred_element_type=f32)
    lax.fori_loop(1, NG, qproj_body, None)
    with ns("pe_scatter"):
        scatter()

    def head_body(n, _):
        @pl.when(n + 1 < H // HPB)
        def _():
            for cp in head_cps(n + 1):
                cp.start()
        for cp in head_cps(n):
            cp.wait()
        with ns("pf_attn"):
            _attention([n * HPB + j for j in range(HPB)], q_ref, k_ref.at[n % 2], v_ref.at[n % 2], oh_ref, n < H)
    lax.fori_loop(0, H // HPB, head_body, None)

    def out_cp(i):
        rows = pl.ds(pl.multiple_of(i * OB, OB), OB)
        return pltpu.make_async_copy(res_ref.at[rows], out_hbm.at[rows], out_sem.at[i])

    def out_body(i, _):
        rows = pl.ds(pl.multiple_of(i * OB, OB), OB)
        s, gate = None, []
        for g in range(NG):
            o = [oh_ref[g * HG + j, rows, :] for j in range(HG)]
            if 1 <= g <= D // 128:
                xb = xb_ref[rows, (g - 1) * 128:g * 128].astype(f32)
                gate.append((xb * _sigmoid(xb)).astype(bf16))
                o[0] = jnp.where(i < S, o[0], gate[-1])
            d = jnp.dot(jnp.concatenate(o, axis=1), wo_ref[g * cw:(g + 1) * cw, :], preferred_element_type=f32)
            s = d if s is None else s + d
        gate = jnp.concatenate(gate, axis=1).astype(f32)
        res_ref[rows, :] = (x_ref[rows, :].astype(f32) + s * gate).astype(bf16)
        out_cp(i).start()
    with ns("pg_out"):
        lax.fori_loop(0, S // OB, out_body, None)
    with ns("ph_wait"):
        for i in range(S // OB):
            out_cp(i).wait()


@jax.jit
def pallas_recurrent_scan__mha_block_cached__moe_arch_mod__prompt_kernel(
        A_x, A_k_cache, A_v_cache, A_wq, A_wo, B_x, B_w_r, B_w_gate, B_w_up, B_w_down):
    hbm = pl.BlockSpec(memory_space=pltpu.HBM)
    vm = pltpu.VMEM
    dma = pltpu.SemaphoreType.DMA
    out = pl.pallas_call(
        _kernel,
        in_specs=[hbm] * 9,
        out_specs=hbm,
        out_shape=jax.ShapeDtypeStruct((S, D), bf16),
        scratch_shapes=[
            vm((S, D), bf16), vm((2, HPB, S, DH), bf16), vm((2, HPB, S, DH), bf16), vm((NG, D, HG * DH), bf16),
            vm((H * DH, D), bf16), vm((D,), bf16), vm((NG - 1, 2 * FP, D), bf16), vm((NG - 1, FP, D), bf16),
            vm((S, D), bf16), vm((S, D), bf16), vm((S // 128, 128), f32), vm((H, S, DH), bf16), vm((H, S, DH), bf16),
            vm((S, D), bf16), pltpu.SMEM((C,), i32), vm((16, D), bf16), vm((C, 128), f32), vm((16, D), f32),
            dma((len(X_PIECES),)), dma, dma((4, NG)), dma((3, H // HPB)), dma((S // OB,)),
        ],
        compiler_params=pltpu.CompilerParams(vmem_limit_bytes=100 * 2**20, disable_bounds_checks=True),
    )(A_x.reshape(S, D), A_k_cache.reshape(H, S, DH), A_v_cache.reshape(H, S, DH), A_wq, A_wo,
      B_w_r, B_w_gate.T, B_w_up.T, B_w_down)
    return out.reshape(1, S, D)
```

```python
import contextlib
import jax
import jax.numpy as jnp
import ml_dtypes
import numpy as np
from jax import lax
import jax.experimental.pallas as pl
import jax.experimental.pallas.tpu as pltpu

S, D, H, DH, F, C = 2048, 640, 32, 128, 1728, 8
BP = 256
LEAD = 160
T0 = 0
AT = 0
MODE = 2
CK = 512
RB = 256
HG = 4
NG = H // HG
OB = 288
HPB = 2
FP = 256
PROF = 0
bf16, f32, i32 = jnp.bfloat16, jnp.float32, jnp.int32
NT = (((1,), (1,)), ((), ()))
QSCALE = float(DH ** -0.5 * np.log2(np.e))
EPS = float(np.asarray(1e-5, ml_dtypes.bfloat16))
KEY_BASE = 0x20000000
X_PIECES = ((0, 256), (256, 256), (512, 512), (1024, 1024))


def ns(name):
    return jax.named_scope(name) if PROF else contextlib.nullcontext()


def _round(v):
    return v.astype(bf16).astype(f32)


def _sigmoid(v):
    return 1.0 / (1.0 + jnp.exp(-v))


def _attention(heads, q_ref, k_ref, v_ref, o_ref, always):
    nc, nt = S // CK, CK // 128
    scores, run_max, row_max, run_sum, acc = {}, {}, {}, {}, {}
    pace = []

    def qk(h, c):
        s = lax.dot_general(q_ref[heads[h]], k_ref[h, c * CK:(c + 1) * CK, :], NT, preferred_element_type=f32)
        scores[h, c] = s
        m = run_max.get(h)
        for t in range(nt):
            st = s[:, t * 128:(t + 1) * 128]
            m = st if m is None else jnp.maximum(m, st)
        run_max[h] = m
        if c == nc - 1:
            row_max[h] = jnp.broadcast_to(jnp.max(m, axis=-1, keepdims=True), (S, 128))

    def pv(h, j, c):
        rows = slice(j * BP, (j + 1) * BP)
        if not pace:
            tail = scores[1, 0 if MODE == 0 else nc - 1][S - LEAD:, T0 * 128:(T0 + 1) * 128]
            pace.append(jnp.concatenate([tail] + [tail[LEAD - 8:]] * ((BP - LEAD) // 8), axis=0))
        m = jnp.where(always, row_max[h][rows], pace.pop())
        s = scores[h, c][rows]
        ps = [jnp.exp2(s[:, t * 128:(t + 1) * 128] - m) for t in range(nt)]
        l = run_sum.get((h, j))
        for pt in ps:
            l = pt if l is None else l + pt
        run_sum[h, j] = l
        ps[AT] = jnp.where(always, ps[AT], l)
        p = jnp.concatenate(ps, axis=1).astype(bf16)
        d = jnp.dot(p, v_ref[h, c * CK:(c + 1) * CK, :], preferred_element_type=f32)
        o = d if c == 0 else acc[h, j] + d
        acc[h, j] = o
        if c == nc - 1:
            lr = jnp.sum(l, axis=-1, keepdims=True)
            r = pl.reciprocal(lr, approx=True)
            o = o * (r * (2.0 - lr * r))
            o_ref[heads[h], rows, :] = o.astype(bf16)
        pace.append(o)

    tasks = [(j, c) for j in range(S // BP) for c in range(nc)]
    per = len(tasks) // nc
    for c in range(nc):
        qk(0, c)
    for h in range(len(heads)):
        for c in range(nc):
            if h + 1 < len(heads):
                for cc in ([c] if MODE == 0 else range(nc) if c == 0 else ()):
                    qk(h + 1, cc)
            for j, cc in tasks[c * per:(c + 1) * per]:
                pv(h, j, cc)


def _kernel(x_hbm, k_hbm, v_hbm, wq_hbm, wo_hbm, wr_hbm, wg_hbm, wu_hbm, wd_hbm, out_hbm,
            x_ref, k_ref, v_ref, wq_ref, wo_ref, wr_ref, wgu_ref, wd_ref,
            xn_ref, r_ref, q_ref, oh_ref, res_ref, idx_ref, xsel_ref, rsel_ref, y_ref,
            x_sem, wr_sem, w_sem, kv_sem, out_sem):
    cw = HG * DH
    x_cp = [pltpu.make_async_copy(x_hbm.at[pl.ds(a, n)], x_ref.at[pl.ds(a, n)], x_sem.at[j])
            for j, (a, n) in enumerate(X_PIECES)]
    wr_cp = pltpu.make_async_copy(wr_hbm, wr_ref, wr_sem)

    def wq_cp(g):
        cols = g * cw if isinstance(g, int) else pl.multiple_of(g * cw, cw)
        return pltpu.make_async_copy(wq_hbm.at[:, pl.ds(cols, cw)], wq_ref.at[g], w_sem.at[0, g])

    def ffn_start(g):
        return min((g - 1) * FP, F - FP) if isinstance(g, int) else pl.multiple_of(jnp.minimum((g - 1) * FP, F - FP), 16)

    def chunk_cps(g):
        rows = pl.ds(ffn_start(g), FP)
        return (wq_cp(g),
                pltpu.make_async_copy(wg_hbm.at[rows], wgu_ref.at[g - 1, pl.ds(0, FP)], w_sem.at[1, g]),
                pltpu.make_async_copy(wu_hbm.at[rows], wgu_ref.at[g - 1, pl.ds(FP, FP)], w_sem.at[2, g]),
                pltpu.make_async_copy(wd_hbm.at[rows], wd_ref.at[g - 1], w_sem.at[3, g]))

    def head_cps(n):
        hs = pl.ds(n * HPB, HPB)
        wo_rows = pl.ds(pl.multiple_of(n * HPB * DH, DH), HPB * DH)
        return (pltpu.make_async_copy(k_hbm.at[hs], k_ref.at[n % 2], kv_sem.at[0, n]),
                pltpu.make_async_copy(v_hbm.at[hs], v_ref.at[n % 2], kv_sem.at[1, n]),
                pltpu.make_async_copy(wo_hbm.at[wo_rows], wo_ref.at[wo_rows], kv_sem.at[2, n]))

    def layernorm(r0, n=RB):
        rows = slice(r0, r0 + n)
        x = x_ref[rows, :].astype(f32)
        mean = jnp.sum(x, axis=-1, keepdims=True) * (1.0 / D)
        xc = x - mean
        var = jnp.sum(xc * xc, axis=-1, keepdims=True) * (1.0 / D)
        var = _round(_round(var) + EPS)
        rs = lax.rsqrt(var)
        den = _round(var * rs)
        xn32 = xc * (rs * (2.0 - den * rs))
        xn = xn32.astype(bf16)
        xn_ref[rows, :] = xn
        r = jnp.sum(xn32 * wr_ref[...].astype(f32).reshape(1, D), axis=-1, keepdims=True)
        eye = lax.broadcasted_iota(i32, (128, 128), 0) == lax.broadcasted_iota(i32, (128, 128), 1)
        for j in range(n // 128):
            g = r0 // 128 + j
            r_ref[g:g + 1, :] = jnp.sum(jnp.where(eye, r[j * 128:(j + 1) * 128], 0.0), axis=0, keepdims=True)

    def qproj(r0, g, n=RB):
        rows = slice(r0, r0 + n)
        q = jnp.dot(xn_ref[rows, :], wq_ref[g], preferred_element_type=f32) * QSCALE
        for j in range(HG):
            q_ref[g * HG + j, rows, :] = q[:, j * DH:(j + 1) * DH].astype(bf16)

    def select_tokens():
        r = _round(r_ref[...])
        pos = lax.broadcasted_iota(i32, r.shape, 0) * 128 + lax.broadcasted_iota(i32, r.shape, 1)
        b = lax.shift_right_logical(pltpu.bitcast(jnp.where(r == 0.0, 0.0, r), i32), 16)
        u = jnp.where(b < 0x8000, b + 0x8000, 0xFFFF - b)
        u = jnp.where(r != r, 0, u)
        key = pltpu.bitcast(KEY_BASE + u * S + (S - 1 - pos), f32)
        sub8 = lax.broadcasted_iota(i32, (C, 128), 0)
        top_all = jnp.zeros((C, 128), f32)
        for c in range(C):
            top = jnp.max(jnp.max(key, axis=0, keepdims=True), axis=1, keepdims=True)
            key = jnp.where(key == top, 0.0, key)
            top_all = jnp.where(sub8 == c, top, top_all)
        bits = pltpu.bitcast(top_all, i32) - KEY_BASE
        u = lax.shift_right_logical(bits, 11)
        b = jnp.where(u >= 0x8000, u - 0x8000, 0xFFFF - u)
        rsel_ref[...] = _sigmoid(pltpu.bitcast(lax.shift_left(b, 16), f32))
        idx = (S - 1) - (bits & (S - 1))
        sub16 = lax.broadcasted_iota(i32, (16, D), 0)
        xsel = jnp.zeros((16, D), f32)
        for c in range(C):
            t = idx[c, 0]
            idx_ref[c] = t
            blk = xn_ref[pl.ds(pl.multiple_of(t & ~15, 16), 16), :].astype(f32)
            row = jnp.sum(jnp.where(sub16 == (t & 15), blk, 0.0), axis=0, keepdims=True)
            xsel = jnp.where(sub16 == c, row, xsel)
        xsel_ref[...] = xsel.astype(bf16)
        y_ref[...] = jnp.zeros_like(y_ref)

    def scatter():
        y = _round(y_ref[:C, :] * rsel_ref[:, :1])
        sub16 = lax.broadcasted_iota(i32, (16, D), 0)
        for c in range(C):
            t = idx_ref[c]
            rows = pl.ds(pl.multiple_of(t & ~15, 16), 16)
            blk = xn_ref[rows, :].astype(f32)
            xn_ref[rows, :] = jnp.where(sub16 == (t & 15), blk + y[c:c + 1], blk).astype(bf16)

    nrb = S // RB
    with ns("p0_start"):
        x_cp[0].start(); wr_cp.start(); wq_cp(0).start()
        x_cp[0].wait(); wr_cp.wait()
        x_cp[1].start()
    with ns("p1_ln0"):
        layernorm(0)
    with ns("p2_wait"):
        wq_cp(0).wait()
        x_cp[2].start()
    with ns("p3a"):
        qproj(0, 0, 128)
    with ns("p3a_wait"):
        x_cp[1].wait()
        x_cp[3].start()
    with ns("p3b"):
        layernorm(256); qproj(128, 0, 128)
    with ns("p4_wait"):
        x_cp[2].wait()
        for cp in chunk_cps(1):
            cp.start()
    with ns("p5"):
        layernorm(512); qproj(256, 0); layernorm(768); qproj(512, 0)
    with ns("p6_wait"):
        x_cp[3].wait()
    with ns("p7"):
        layernorm(1024); qproj(768, 0); layernorm(1280); qproj(1024, 0); layernorm(1536); layernorm(1792); qproj(1280, 0)
        select_tokens()
        qproj(1536, 0); qproj(1792, 0)

    def qproj_body(g, _):
        @pl.when(g + 1 < NG)
        def _():
            for cp in chunk_cps(g + 1):
                cp.start()

        @pl.when(g + 1 == NG)
        def _():
            for cp in head_cps(0):
                cp.start()
        for cp in chunk_cps(g):
            cp.wait()
        with ns("pd_q"):
            au = None
            for rb in range(nrb):
                qproj(rb * RB, g)
                if rb < D // 128:
                    cols = slice(rb * 128, (rb + 1) * 128)
                    d = lax.dot_general(xsel_ref[:, cols], wgu_ref[g - 1, :, cols], NT, preferred_element_type=f32)
                    au = d if au is None else au + d
                elif rb == D // 128:
                    a, u = au[:, :FP], au[:, FP:]
                    fresh = lax.broadcasted_iota(i32, (16, FP), 1) >= (g - 1) * FP - ffn_start(g)
                    hid = jnp.where(fresh, a * _sigmoid(a) * u, 0.0).astype(bf16)
                    y_ref[...] += jnp.dot(hid, wd_ref[g - 1], preferred_element_type=f32)
    lax.fori_loop(1, NG, qproj_body, None)
    with ns("pe_scatter"):
        scatter()

    def head_body(n, _):
        @pl.when(n + 1 < H // HPB)
        def _():
            for cp in head_cps(n + 1):
                cp.start()
        for cp in head_cps(n):
            cp.wait()
        with ns("pf_attn"):
            _attention([n * HPB + j for j in range(HPB)], q_ref, k_ref.at[n % 2], v_ref.at[n % 2], oh_ref, n < H)
    lax.fori_loop(0, H // HPB, head_body, None)

    def out_cp(i, n):
        rows = pl.ds(i * OB if isinstance(i, int) else pl.multiple_of(i * OB, 16), n)
        return pltpu.make_async_copy(res_ref.at[rows], out_hbm.at[rows], out_sem.at[i])

    def out_block(i, n):
        r0 = i * OB if isinstance(i, int) else pl.multiple_of(i * OB, 16)
        rows = pl.ds(r0, n)
        s, gate = None, []
        for g in range(NG):
            o = [oh_ref[g * HG + j, rows, :] for j in range(HG)]
            if 1 <= g <= D // 128:
                cols = slice((g - 1) * 128, g * 128)
                xb = xn_ref[rows, cols].astype(f32)
                gate.append((xb * _sigmoid(xb)).astype(bf16))
                o[0] = jnp.where(idx_ref[0] >= 0 if isinstance(i, int) else i < S, o[0], gate[-1])
            d = jnp.dot(jnp.concatenate(o, axis=1), wo_ref[g * cw:(g + 1) * cw, :], preferred_element_type=f32)
            s = d if s is None else s + d
        gate = jnp.concatenate(gate, axis=1).astype(f32)
        res_ref[rows, :] = (x_ref[rows, :].astype(f32) + s * gate).astype(bf16)
        out_cp(i, n).start()

    nob = S // OB
    with ns("pg_out"):
        lax.fori_loop(0, nob, lambda i, _: out_block(i, OB), None)
        if S % OB:
            out_block(nob, S % OB)
    with ns("ph_wait"):
        for i in range(nob):
            out_cp(i, OB).wait()
        if S % OB:
            out_cp(nob, S % OB).wait()


@jax.jit
def pallas_recurrent_scan__mha_block_cached__moe_arch_mod__prompt_kernel(
        A_x, A_k_cache, A_v_cache, A_wq, A_wo, B_x, B_w_r, B_w_gate, B_w_up, B_w_down):
    hbm = pl.BlockSpec(memory_space=pltpu.HBM)
    vm = pltpu.VMEM
    dma = pltpu.SemaphoreType.DMA
    out = pl.pallas_call(
        _kernel,
        in_specs=[hbm] * 9,
        out_specs=hbm,
        out_shape=jax.ShapeDtypeStruct((S, D), bf16),
        scratch_shapes=[
            vm((S, D), bf16), vm((2, HPB, S, DH), bf16), vm((2, HPB, S, DH), bf16), vm((NG, D, HG * DH), bf16),
            vm((H * DH, D), bf16), vm((D,), bf16), vm((NG - 1, 2 * FP, D), bf16), vm((NG - 1, FP, D), bf16),
            vm((S, D), bf16), vm((S // 128, 128), f32), vm((H, S, DH), bf16), vm((H, S, DH), bf16),
            vm((S, D), bf16), pltpu.SMEM((C,), i32), vm((16, D), bf16), vm((C, 128), f32), vm((16, D), f32),
            dma((len(X_PIECES),)), dma, dma((4, NG)), dma((3, H // HPB)), dma((pl.cdiv(S, OB),)),
        ],
        compiler_params=pltpu.CompilerParams(vmem_limit_bytes=120 * 2**20, disable_bounds_checks=True),
    )(A_x.reshape(S, D), A_k_cache.reshape(H, S, DH), A_v_cache.reshape(H, S, DH), A_wq, A_wo,
      B_w_r, B_w_gate.T, B_w_up.T, B_w_down)
    return out.reshape(1, S, D)
```

```python
import jax
import jax.numpy as jnp
import ml_dtypes
import numpy as np
from jax import lax
import jax.experimental.pallas as pl
import jax.experimental.pallas.tpu as pltpu

S, D, H, DH, F, C = 2048, 640, 32, 128, 1728, 8
CK = 4 * 128
BP = 256
LEAD = 160
HPB = 2
RB = 256
HG = 4
NG = H // HG
FP = 256
OB = 288
X_PIECES = ((0, 256), (256, 256), (512, 512), (1024, 1024))

bf16, f32, i32 = jnp.bfloat16, jnp.float32, jnp.int32
NT = (((1,), (1,)), ((), ()))
QSCALE = float(DH ** -0.5 * np.log2(np.e))
EPS = float(np.asarray(1e-5, ml_dtypes.bfloat16))
F32_MAX = float(np.finfo(np.float32).max)
KEY_BASE = 0x20000000


def _round(v):
    return v.astype(bf16).astype(f32)


def _sigmoid(v):
    return 1.0 / (1.0 + jnp.exp(-v))


def _attention(heads, q_ref, k_ref, v_ref, o_ref, always):
    nc = S // CK
    scores, row_max = {}, {}
    for h, head in enumerate(heads):
        m = None
        for c in range(nc):
            s = lax.dot_general(q_ref[head], k_ref[h, c * CK:(c + 1) * CK, :], NT, preferred_element_type=f32)
            scores[h, c] = s
            for t in range(0, CK, 128):
                m = s[:, t:t + 128] if m is None else jnp.maximum(m, s[:, t:t + 128])
        row_max[h] = jnp.broadcast_to(jnp.max(m, axis=-1, keepdims=True), (S, 128))

    tail = s[S - LEAD:, :128]
    pace = jnp.concatenate([tail] + [tail[LEAD - 8:]] * ((BP - LEAD) // 8), axis=0)
    for h, head in enumerate(heads):
        for r0 in range(0, S, BP):
            rows = slice(r0, r0 + BP)
            l = o = None
            for c in range(nc):
                m = jnp.where(always, row_max[h][rows], pace)
                s = scores[h, c][rows]
                p = [jnp.exp2(s[:, t:t + 128] - m) for t in range(0, CK, 128)]
                t = (p[0] + p[1]) + (p[2] + p[3])
                l = t if l is None else l + t
                p[0] = jnp.where(always, p[0], l)
                d = jnp.dot(jnp.concatenate(p, axis=1).astype(bf16), v_ref[h, c * CK:(c + 1) * CK, :],
                            preferred_element_type=f32)
                o = d if o is None else o + d
                pace = o
            l = jnp.sum(l, axis=-1, keepdims=True)
            r = pl.reciprocal(l, approx=True)
            pace = o = o * (r * (2.0 - l * r))
            o_ref[head, rows, :] = o.astype(bf16)


def _kernel(x_hbm, k_hbm, v_hbm, wq_hbm, wo_hbm, wr_hbm, wg_hbm, wu_hbm, wd_hbm, out_hbm,
            x_ref, k_ref, v_ref, wq_ref, wo_ref, wr_ref, wgu_ref, wd_ref,
            xn_ref, r_ref, q_ref, oh_ref, res_ref, idx_ref, xsel_ref, rsel_ref, y_ref,
            x_sem, wr_sem, w_sem, kv_sem, out_sem):
    cw = HG * DH

    def aligned(i, n):
        return i if isinstance(i, int) else pl.multiple_of(i, n)

    x_cp = [pltpu.make_async_copy(x_hbm.at[pl.ds(a, n)], x_ref.at[pl.ds(a, n)], x_sem.at[j])
            for j, (a, n) in enumerate(X_PIECES)]
    wr_cp = pltpu.make_async_copy(wr_hbm, wr_ref, wr_sem)

    def wq_cp(g):
        return pltpu.make_async_copy(wq_hbm.at[:, pl.ds(aligned(g * cw, cw), cw)], wq_ref.at[g], w_sem.at[0, g])

    def ffn_start(g):
        return min((g - 1) * FP, F - FP) if isinstance(g, int) else jnp.minimum((g - 1) * FP, F - FP)

    def chunk_cps(g):
        rows = pl.ds(aligned(ffn_start(g), 16), FP)
        return (wq_cp(g),
                pltpu.make_async_copy(wg_hbm.at[rows], wgu_ref.at[g - 1, pl.ds(0, FP)], w_sem.at[1, g]),
                pltpu.make_async_copy(wu_hbm.at[rows], wgu_ref.at[g - 1, pl.ds(FP, FP)], w_sem.at[2, g]),
                pltpu.make_async_copy(wd_hbm.at[rows], wd_ref.at[g - 1], w_sem.at[3, g]))

    def head_cps(n):
        hs = pl.ds(n * HPB, HPB)
        wo_rows = pl.ds(aligned(n * HPB * DH, DH), HPB * DH)
        return (pltpu.make_async_copy(k_hbm.at[hs], k_ref.at[n % 2], kv_sem.at[0, n]),
                pltpu.make_async_copy(v_hbm.at[hs], v_ref.at[n % 2], kv_sem.at[1, n]),
                pltpu.make_async_copy(wo_hbm.at[wo_rows], wo_ref.at[wo_rows], kv_sem.at[2, n]))

    def out_cp(i, n):
        rows = pl.ds(aligned(i * OB, 16), n)
        return pltpu.make_async_copy(res_ref.at[rows], out_hbm.at[rows], out_sem.at[i])

    def layernorm(r0):
        rows = slice(r0, r0 + RB)
        x = x_ref[rows, :].astype(f32)
        xc = x - jnp.sum(x, axis=-1, keepdims=True) * (1.0 / D)
        var = jnp.sum(xc * xc, axis=-1, keepdims=True) * (1.0 / D)
        var = _round(_round(var) + EPS)
        rs = lax.rsqrt(var)
        den = _round(jnp.minimum(var, F32_MAX) * rs)
        xn = xc * (rs * (2.0 - den * rs))
        xn_ref[rows, :] = xn.astype(bf16)
        r = jnp.sum(xn * wr_ref[...].astype(f32).reshape(1, D), axis=-1, keepdims=True)
        eye = lax.broadcasted_iota(i32, (128, 128), 0) == lax.broadcasted_iota(i32, (128, 128), 1)
        for j in range(0, RB, 128):
            g = (r0 + j) // 128
            r_ref[g:g + 1, :] = jnp.sum(jnp.where(eye, r[j:j + 128], 0.0), axis=0, keepdims=True)

    def qproj(r0, g, n=RB):
        rows = slice(r0, r0 + n)
        q = jnp.dot(xn_ref[rows, :], wq_ref[g], preferred_element_type=f32) * QSCALE
        for j in range(HG):
            q_ref[g * HG + j, rows, :] = q[:, j * DH:(j + 1) * DH].astype(bf16)

    def select_tokens():
        r = _round(r_ref[...])
        pos = lax.broadcasted_iota(i32, r.shape, 0) * 128 + lax.broadcasted_iota(i32, r.shape, 1)
        b = lax.shift_right_logical(pltpu.bitcast(jnp.where(r == 0.0, 0.0, r), i32), 16)
        u = jnp.where(b < 0x8000, b + 0x8000, 0xFFFF - b)
        u = jnp.where(r != r, 0, u)
        key = pltpu.bitcast(KEY_BASE + u * S + (S - 1 - pos), f32)
        sub8 = lax.broadcasted_iota(i32, (C, 128), 0)
        top_all = jnp.zeros((C, 128), f32)
        for c in range(C):
            top = jnp.max(jnp.max(key, axis=0, keepdims=True), axis=1, keepdims=True)
            key = jnp.where(key == top, 0.0, key)
            top_all = jnp.where(sub8 == c, top, top_all)
        bits = pltpu.bitcast(top_all, i32) - KEY_BASE
        u = lax.shift_right_logical(bits, S.bit_length() - 1)
        b = jnp.where(u >= 0x8000, u - 0x8000, 0xFFFF - u)
        rsel_ref[...] = _sigmoid(pltpu.bitcast(lax.shift_left(b, 16), f32))
        idx = (S - 1) - (bits & (S - 1))
        sub16 = lax.broadcasted_iota(i32, (16, D), 0)
        xsel = jnp.zeros((16, D), f32)
        for c in range(C):
            t = jnp.clip(idx[c, 0], 0, S - 1)
            idx_ref[c] = t
            blk = xn_ref[pl.ds(pl.multiple_of(t & ~15, 16), 16), :].astype(f32)
            row = jnp.sum(jnp.where(sub16 == (t & 15), blk, 0.0), axis=0, keepdims=True)
            xsel = jnp.where(sub16 == c, row, xsel)
        xsel_ref[...] = xsel.astype(bf16)
        y_ref[...] = jnp.zeros_like(y_ref)

    def scatter():
        y = _round(y_ref[:C, :] * rsel_ref[:, :1])
        sub16 = lax.broadcasted_iota(i32, (16, D), 0)
        for c in range(C):
            t = jnp.clip(idx_ref[c], 0, S - 1)
            rows = pl.ds(pl.multiple_of(t & ~15, 16), 16)
            blk = xn_ref[rows, :].astype(f32)
            xn_ref[rows, :] = jnp.where(sub16 == (t & 15), blk + y[c:c + 1], blk).astype(bf16)

    x_cp[0].start(); wr_cp.start(); wq_cp(0).start()
    x_cp[0].wait(); wr_cp.wait()
    x_cp[1].start()
    layernorm(0)
    wq_cp(0).wait()
    x_cp[2].start()
    qproj(0, 0, 128)
    x_cp[1].wait()
    x_cp[3].start()
    layernorm(256); qproj(128, 0, 128)
    x_cp[2].wait()
    for cp in chunk_cps(1):
        cp.start()
    layernorm(512); qproj(256, 0); layernorm(768); qproj(512, 0)
    x_cp[3].wait()
    layernorm(1024); qproj(768, 0); layernorm(1280); qproj(1024, 0)
    layernorm(1536); layernorm(1792); qproj(1280, 0)
    select_tokens()
    qproj(1536, 0); qproj(1792, 0)

    def qproj_body(g, _):
        @pl.when(g + 1 < NG)
        def _():
            for cp in chunk_cps(g + 1):
                cp.start()

        @pl.when(g + 1 == NG)
        def _():
            for cp in head_cps(0):
                cp.start()

        for cp in chunk_cps(g):
            cp.wait()
        au = None
        for rb in range(S // RB):
            qproj(rb * RB, g)
            if rb < D // 128:
                cols = slice(rb * 128, (rb + 1) * 128)
                d = lax.dot_general(xsel_ref[:, cols], wgu_ref[g - 1, :, cols], NT, preferred_element_type=f32)
                au = d if au is None else au + d
            elif rb == D // 128:
                a, u = au[:, :FP], au[:, FP:]
                fresh = lax.broadcasted_iota(i32, (16, FP), 1) >= (g - 1) * FP - ffn_start(g)
                hid = jnp.where(fresh, a * _sigmoid(a) * u, 0.0).astype(bf16)
                y_ref[...] += jnp.dot(hid, wd_ref[g - 1], preferred_element_type=f32)

    lax.fori_loop(1, NG, qproj_body, None)
    scatter()

    def head_body(n, _):
        @pl.when(n + 1 < H // HPB)
        def _():
            for cp in head_cps(n + 1):
                cp.start()

        for cp in head_cps(n):
            cp.wait()
        _attention([n * HPB + j for j in range(HPB)], q_ref, k_ref.at[n % 2], v_ref.at[n % 2], oh_ref, n < H)

    lax.fori_loop(0, H // HPB, head_body, None)

    def out_block(i, n, always):
        rows = pl.ds(aligned(i * OB, 16), n)
        s, gate = None, []
        for g in range(NG):
            o = [oh_ref[g * HG + j, rows, :] for j in range(HG)]
            if 1 <= g <= D // 128:
                xb = xn_ref[rows, (g - 1) * 128:g * 128].astype(f32)
                gate.append((xb * _sigmoid(xb)).astype(bf16))
                o[0] = jnp.where(always, o[0], gate[-1])
            d = jnp.dot(jnp.concatenate(o, axis=1), wo_ref[g * cw:(g + 1) * cw, :], preferred_element_type=f32)
            s = d if s is None else s + d
        gate = jnp.concatenate(gate, axis=1).astype(f32)
        res_ref[rows, :] = (x_ref[rows, :].astype(f32) + s * gate).astype(bf16)
        out_cp(i, n).start()

    nob = S // OB
    lax.fori_loop(0, nob, lambda i, _: out_block(i, OB, i < S), None)
    out_block(nob, S % OB, idx_ref[0] >= 0)
    for i in range(nob):
        out_cp(i, OB).wait()
    out_cp(nob, S % OB).wait()


@jax.jit
def pallas_recurrent_scan__mha_block_cached__moe_arch_mod__prompt_kernel(
    A_x: jax.Array,
    A_k_cache: jax.Array,
    A_v_cache: jax.Array,
    A_wq: jax.Array,
    A_wo: jax.Array,
    B_x: jax.Array,
    B_w_r: jax.Array,
    B_w_gate: jax.Array,
    B_w_up: jax.Array,
    B_w_down: jax.Array,
):
    del B_x
    hbm = pl.BlockSpec(memory_space=pltpu.HBM)
    vm = pltpu.VMEM
    dma = pltpu.SemaphoreType.DMA
    out = pl.pallas_call(
        _kernel,
        in_specs=[hbm] * 9,
        out_specs=hbm,
        out_shape=jax.ShapeDtypeStruct((S, D), bf16),
        scratch_shapes=[
            vm((S, D), bf16),
            vm((2, HPB, S, DH), bf16),
            vm((2, HPB, S, DH), bf16),
            vm((NG, D, HG * DH), bf16),
            vm((H * DH, D), bf16),
            vm((D,), bf16),
            vm((NG - 1, 2 * FP, D), bf16),
            vm((NG - 1, FP, D), bf16),
            vm((S, D), bf16),
            vm((S // 128, 128), f32),
            vm((H, S, DH), bf16),
            vm((H, S, DH), bf16),
            vm((S, D), bf16),
            pltpu.SMEM((C,), i32),
            vm((16, D), bf16),
            vm((C, 128), f32),
            vm((16, D), f32),
            dma((len(X_PIECES),)), dma, dma((4, NG)), dma((3, H // HPB)), dma((S // OB + 1,)),
        ],
        compiler_params=pltpu.CompilerParams(vmem_limit_bytes=120 * 2**20, disable_bounds_checks=True),
    )(A_x.reshape(S, D), A_k_cache.reshape(H, S, DH), A_v_cache.reshape(H, S, DH), A_wq, A_wo,
      B_w_r, B_w_gate.T, B_w_up.T, B_w_down)
    return out.reshape(1, S, D)
```

```python
import jax
import jax.numpy as jnp
import ml_dtypes
import numpy as np
from jax import lax
import jax.experimental.pallas as pl
import jax.experimental.pallas.tpu as pltpu

S, D, H, DH, F, C = 2048, 640, 32, 128, 1728, 8
CK = 4 * 128
BP = 256
LEAD = 160
HPB = 2
RB = 256
HG = 4
NG = H // HG
FP = 256
OB = 288
X_PIECES = ((0, 256), (256, 256), (512, 512), (1024, 1024))

bf16, f32, i32 = jnp.bfloat16, jnp.float32, jnp.int32
NT = (((1,), (1,)), ((), ()))
QSCALE = float(DH ** -0.5 * np.log2(np.e))
EPS = float(np.asarray(1e-5, ml_dtypes.bfloat16))
F32_MAX = float(np.finfo(np.float32).max)
KEY_BASE = 0x20000000


def _round(v):
    return v.astype(bf16).astype(f32)


def _sigmoid(v):
    return 1.0 / (1.0 + jnp.exp(-v))


def _attention(heads, q_ref, k_ref, v_ref, o_ref, always):
    nc = S // CK
    scores, row_max = {}, {}
    for h, head in enumerate(heads):
        m = None
        for c in range(nc):
            s = lax.dot_general(q_ref[head], k_ref[h, c * CK:(c + 1) * CK, :], NT, preferred_element_type=f32)
            scores[h, c] = s
            for t in range(0, CK, 128):
                m = s[:, t:t + 128] if m is None else jnp.maximum(m, s[:, t:t + 128])
        row_max[h] = jnp.broadcast_to(jnp.max(m, axis=-1, keepdims=True), (S, 128))

    tail = s[S - LEAD:, :128]
    pace = jnp.concatenate([tail] + [tail[LEAD - 8:]] * ((BP - LEAD) // 8), axis=0)
    for h, head in enumerate(heads):
        for r0 in range(0, S, BP):
            rows = slice(r0, r0 + BP)
            l = o = None
            for c in range(nc):
                m = jnp.where(always, row_max[h][rows], pace)
                s = scores[h, c][rows]
                p = [jnp.exp2(s[:, t:t + 128] - m) for t in range(0, CK, 128)]
                t = (p[0] + p[1]) + (p[2] + p[3])
                l = t if l is None else l + t
                p[0] = jnp.where(always, p[0], l)
                d = jnp.dot(jnp.concatenate(p, axis=1).astype(bf16), v_ref[h, c * CK:(c + 1) * CK, :],
                            preferred_element_type=f32)
                o = d if o is None else o + d
                pace = o
            l = jnp.sum(l, axis=-1, keepdims=True)
            r = pl.reciprocal(l, approx=True)
            pace = o = o * (r * (2.0 - l * r))
            o_ref[head, rows, :] = o.astype(bf16)


def _kernel(x_hbm, k_hbm, v_hbm, wq_hbm, wo_hbm, wr_hbm, wg_hbm, wu_hbm, wd_hbm, out_hbm,
            x_ref, k_ref, v_ref, wq_ref, wo_ref, wr_ref, wgu_ref, wd_ref,
            xn_ref, r_ref, q_ref, oh_ref, res_ref, idx_ref, xsel_ref, rsel_ref, y_ref,
            x_sem, wr_sem, wo_sem, w_sem, kv_sem, out_sem):
    cw = HG * DH

    def aligned(i, n):
        return i if isinstance(i, int) else pl.multiple_of(i, n)

    x_cp = [pltpu.make_async_copy(x_hbm.at[pl.ds(a, n)], x_ref.at[pl.ds(a, n)], x_sem.at[j])
            for j, (a, n) in enumerate(X_PIECES)]
    wr_cp = pltpu.make_async_copy(wr_hbm, wr_ref, wr_sem)
    wo_cp = pltpu.make_async_copy(wo_hbm, wo_ref, wo_sem)

    def wq_cp(g):
        return pltpu.make_async_copy(wq_hbm.at[:, pl.ds(aligned(g * cw, cw), cw)], wq_ref.at[g], w_sem.at[0, g])

    def ffn_start(g):
        return min((g - 1) * FP, F - FP) if isinstance(g, int) else jnp.minimum((g - 1) * FP, F - FP)

    def chunk_cps(g):
        rows = pl.ds(aligned(ffn_start(g), 16), FP)
        return (wq_cp(g),
                pltpu.make_async_copy(wg_hbm.at[rows], wgu_ref.at[g - 1, pl.ds(0, FP)], w_sem.at[1, g]),
                pltpu.make_async_copy(wu_hbm.at[rows], wgu_ref.at[g - 1, pl.ds(FP, FP)], w_sem.at[2, g]),
                pltpu.make_async_copy(wd_hbm.at[rows], wd_ref.at[g - 1], w_sem.at[3, g]))

    def head_cps(n):
        hs = pl.ds(n * HPB, HPB)
        return (pltpu.make_async_copy(k_hbm.at[hs], k_ref.at[n & 1], kv_sem.at[0, n]),
                pltpu.make_async_copy(v_hbm.at[hs], v_ref.at[n & 1], kv_sem.at[1, n]))

    def out_cp(i, n):
        rows = pl.ds(aligned(i * OB, 16), n)
        return pltpu.make_async_copy(res_ref.at[rows], out_hbm.at[rows], out_sem.at[i])

    def layernorm(r0):
        rows = slice(r0, r0 + RB)
        x = x_ref[rows, :].astype(f32)
        xc = x - jnp.sum(x, axis=-1, keepdims=True) * (1.0 / D)
        var = jnp.sum(xc * xc, axis=-1, keepdims=True) * (1.0 / D)
        var = _round(_round(var) + EPS)
        rs = lax.rsqrt(var)
        den = _round(jnp.minimum(var, F32_MAX) * rs)
        xn = xc * (rs * (2.0 - den * rs))
        xn_ref[rows, :] = xn.astype(bf16)
        r = jnp.sum(xn * wr_ref[...].astype(f32).reshape(1, D), axis=-1, keepdims=True)
        eye = lax.broadcasted_iota(i32, (128, 128), 0) == lax.broadcasted_iota(i32, (128, 128), 1)
        for j in range(0, RB, 128):
            g = (r0 + j) // 128
            r_ref[g:g + 1, :] = jnp.sum(jnp.where(eye, r[j:j + 128], 0.0), axis=0, keepdims=True)

    def qproj(r0, g, n=RB):
        rows = slice(r0, r0 + n)
        q = jnp.dot(xn_ref[rows, :], wq_ref[g], preferred_element_type=f32) * QSCALE
        for j in range(HG):
            q_ref[g * HG + j, rows, :] = q[:, j * DH:(j + 1) * DH].astype(bf16)

    def select_tokens():
        r = _round(r_ref[...])
        pos = lax.broadcasted_iota(i32, r.shape, 0) * 128 + lax.broadcasted_iota(i32, r.shape, 1)
        b = lax.shift_right_logical(pltpu.bitcast(jnp.where(r == 0.0, 0.0, r), i32), 16)
        u = jnp.where(b < 0x8000, b + 0x8000, 0xFFFF - b)
        u = jnp.where(r != r, 0, u)
        key = pltpu.bitcast(KEY_BASE + u * S + (S - 1 - pos), f32)
        sub8 = lax.broadcasted_iota(i32, (C, 128), 0)
        top_all = jnp.zeros((C, 128), f32)
        for c in range(C):
            top = jnp.max(jnp.max(key, axis=0, keepdims=True), axis=1, keepdims=True)
            key = jnp.where(key == top, 0.0, key)
            top_all = jnp.where(sub8 == c, top, top_all)
        bits = pltpu.bitcast(top_all, i32) - KEY_BASE
        u = lax.shift_right_logical(bits, S.bit_length() - 1)
        b = jnp.where(u >= 0x8000, u - 0x8000, 0xFFFF - u)
        rsel_ref[...] = _sigmoid(pltpu.bitcast(lax.shift_left(b, 16), f32))
        idx = (S - 1) - (bits & (S - 1))
        sub16 = lax.broadcasted_iota(i32, (16, D), 0)
        xsel = jnp.zeros((16, D), f32)
        for c in range(C):
            t = jnp.clip(idx[c, 0], 0, S - 1)
            idx_ref[c] = t
            blk = xn_ref[pl.ds(pl.multiple_of(t & ~15, 16), 16), :].astype(f32)
            row = jnp.sum(jnp.where(sub16 == (t & 15), blk, 0.0), axis=0, keepdims=True)
            xsel = jnp.where(sub16 == c, row, xsel)
        xsel_ref[...] = xsel.astype(bf16)
        y_ref[...] = jnp.zeros_like(y_ref)

    def scatter():
        y = _round(y_ref[:C, :] * rsel_ref[:, :1])
        sub16 = lax.broadcasted_iota(i32, (16, D), 0)
        for c in range(C):
            t = jnp.clip(idx_ref[c], 0, S - 1)
            rows = pl.ds(pl.multiple_of(t & ~15, 16), 16)
            blk = xn_ref[rows, :].astype(f32)
            xn_ref[rows, :] = jnp.where(sub16 == (t & 15), blk + y[c:c + 1], blk).astype(bf16)

    x_cp[0].start(); wr_cp.start(); wq_cp(0).start()
    x_cp[0].wait(); wr_cp.wait()
    x_cp[1].start()
    layernorm(0)
    wq_cp(0).wait()
    x_cp[2].start()
    qproj(0, 0, 128)
    x_cp[1].wait()
    x_cp[3].start()
    layernorm(256); qproj(128, 0, 128)
    x_cp[2].wait()
    for cp in chunk_cps(1):
        cp.start()
    layernorm(512); qproj(256, 0); layernorm(768); qproj(512, 0)
    x_cp[3].wait()
    layernorm(1024); qproj(768, 0); layernorm(1280); qproj(1024, 0)
    layernorm(1536); layernorm(1792); qproj(1280, 0)
    select_tokens()
    qproj(1536, 0); qproj(1792, 0)

    def qproj_body(g, _):
        @pl.when(g + 1 < NG)
        def _():
            for cp in chunk_cps(g + 1):
                cp.start()

        @pl.when(g + 1 == NG)
        def _():
            for cp in head_cps(0):
                cp.start()

        for cp in chunk_cps(g):
            cp.wait()
        au = None
        for rb in range(S // RB):
            qproj(rb * RB, g)
            if rb < D // 128:
                cols = slice(rb * 128, (rb + 1) * 128)
                d = lax.dot_general(xsel_ref[:, cols], wgu_ref[g - 1, :, cols], NT, preferred_element_type=f32)
                au = d if au is None else au + d
            elif rb == D // 128:
                a, u = au[:, :FP], au[:, FP:]
                fresh = lax.broadcasted_iota(i32, (16, FP), 1) >= (g - 1) * FP - ffn_start(g)
                hid = jnp.where(fresh, a * _sigmoid(a) * u, 0.0).astype(bf16)
                y_ref[...] += jnp.dot(hid, wd_ref[g - 1], preferred_element_type=f32)

    lax.fori_loop(1, NG, qproj_body, None)
    wo_cp.start()
    scatter()

    def head_body(n, _):
        @pl.when(n + 1 < H // HPB)
        def _():
            for cp in head_cps(n + 1):
                cp.start()

        for cp in head_cps(n):
            cp.wait()
        _attention([n * HPB + j for j in range(HPB)], q_ref, k_ref.at[n & 1], v_ref.at[n & 1], oh_ref, n < H)

    lax.fori_loop(0, H // HPB, head_body, None)

    def out_block(i, n, always):
        rows = pl.ds(aligned(i * OB, 16), n)
        s, gate = None, []
        for g in range(NG):
            o = [oh_ref[g * HG + j, rows, :] for j in range(HG)]
            if 1 <= g <= D // 128:
                xb = xn_ref[rows, (g - 1) * 128:g * 128].astype(f32)
                gate.append((xb * _sigmoid(xb)).astype(bf16))
                o[0] = jnp.where(always, o[0], gate[-1])
            d = jnp.dot(jnp.concatenate(o, axis=1), wo_ref[g * cw:(g + 1) * cw, :], preferred_element_type=f32)
            s = d if s is None else s + d
        gate = jnp.concatenate(gate, axis=1).astype(f32)
        res_ref[rows, :] = (x_ref[rows, :].astype(f32) + s * gate).astype(bf16)
        out_cp(i, n).start()

    nob = S // OB
    wo_cp.wait()
    lax.fori_loop(0, nob, lambda i, _: out_block(i, OB, i < S), None)
    out_block(nob, S % OB, idx_ref[0] >= 0)
    for i in range(nob):
        out_cp(i, OB).wait()
    out_cp(nob, S % OB).wait()


@jax.jit
def pallas_recurrent_scan__mha_block_cached__moe_arch_mod__prompt_kernel(
    A_x: jax.Array,
    A_k_cache: jax.Array,
    A_v_cache: jax.Array,
    A_wq: jax.Array,
    A_wo: jax.Array,
    B_x: jax.Array,
    B_w_r: jax.Array,
    B_w_gate: jax.Array,
    B_w_up: jax.Array,
    B_w_down: jax.Array,
):
    del B_x
    hbm = pl.BlockSpec(memory_space=pltpu.HBM)
    vm = pltpu.VMEM
    dma = pltpu.SemaphoreType.DMA
    out = pl.pallas_call(
        _kernel,
        in_specs=[hbm] * 9,
        out_specs=hbm,
        out_shape=jax.ShapeDtypeStruct((S, D), bf16),
        scratch_shapes=[
            vm((S, D), bf16),
            vm((2, HPB, S, DH), bf16),
            vm((2, HPB, S, DH), bf16),
            vm((NG, D, HG * DH), bf16),
            vm((H * DH, D), bf16),
            vm((D,), bf16),
            vm((NG - 1, 2 * FP, D), bf16),
            vm((NG - 1, FP, D), bf16),
            vm((S, D), bf16),
            vm((S // 128, 128), f32),
            vm((H, S, DH), bf16),
            vm((H, S, DH), bf16),
            vm((S, D), bf16),
            pltpu.SMEM((C,), i32),
            vm((16, D), bf16),
            vm((C, 128), f32),
            vm((16, D), f32),
            dma((len(X_PIECES),)), dma, dma, dma((4, NG)), dma((2, H // HPB)), dma((S // OB + 1,)),
        ],
        compiler_params=pltpu.CompilerParams(vmem_limit_bytes=120 * 2**20, disable_bounds_checks=True),
    )(A_x.reshape(S, D), A_k_cache.reshape(H, S, DH), A_v_cache.reshape(H, S, DH), A_wq, A_wo,
      B_w_r, B_w_gate.T, B_w_up.T, B_w_down)
    return out.reshape(1, S, D)
```
